```python
import os as _os
_os.environ.setdefault("JAX_PLATFORMS", "cpu")
import jax
import jax.numpy as jnp

def _softmax(x, axis=-1):
    return jax.nn.softmax(x, axis=axis)
def _gelu(x):
    return jax.nn.gelu(x, approximate=True)
def _silu(x):
    return jax.nn.silu(x)
def _sigmoid(x):
    return jax.nn.sigmoid(x)
def _layernorm(x, axis=-1, eps=1e-5):
    m = jnp.mean(x, axis=axis, keepdims=True)
    v = jnp.var(x, axis=axis, keepdims=True)
    return (x - m) / jnp.sqrt(v + eps)
def _scatter_add(tgt, idx, src, axis=0):
    return tgt.at[idx].add(src)
def _segment_sum(src, seg, n):
    return jax.ops.segment_sum(src, seg, n)
class _Rng:
    def __init__(self, key):
        self._k = key
    def _next(self):
        self._k, sub = jax.random.split(self._k)
        return sub
    def normal(self, shape):
        return jax.random.normal(self._next(), shape, dtype=jnp.bfloat16)
    def randint(self, lo, hi, shape):
        return jax.random.randint(self._next(), shape, lo, hi, dtype=jnp.int32)
    def uniform(self, shape, lo=0.0, hi=1.0):
        return jax.random.uniform(self._next(), shape, jnp.bfloat16, lo, hi)
    def permutation(self, n):
        return jax.random.permutation(self._next(), n)


kernel_name = 'sequential_preLN__sliding_block__dense_activation_relu__prompt'

def setup_inputs():
    _rng = _Rng(jax.random.key(int.from_bytes(__import__("os").urandom(4), "little")))
    _w = (lambda a: (lambda t: t.astype(jnp.bfloat16) if jnp.issubdtype(t.dtype, jnp.floating) else t)(jnp.asarray(a)))
    def _A_setup():
        B, S, D = 1, 2048, 640
        return {
            "x": _w((lambda *s: _rng.normal(s) * 0.05)(B, S, D)),
            "wqkv": _w((lambda *s: _rng.normal(s) * 0.05)(D, 3 * D)),
            "wo": _w((lambda *s: _rng.normal(s) * 0.05)(D, D)),
        }
    _A_in = _A_setup()

    def _B_setup():
        B, S, D, Dff = 1, 2048, 640, 1536
        return {
            "x": _w((lambda *s: _rng.normal(s) * 0.05)(B, S, D)),
            "w1": _w((lambda *s: _rng.normal(s) * 0.05)(D, Dff)),
            "w2": _w((lambda *s: _rng.normal(s) * 0.05)(Dff, D)),
        }
    _B_in = _B_setup()

    return {
        "A_x": _A_in["x"],
        "A_wqkv": _A_in["wqkv"],
        "A_wo": _A_in["wo"],
        "B_x": _B_in["x"],
        "B_w1": _B_in["w1"],
        "B_w2": _B_in["w2"],
    }

def reference(A_x, A_wqkv, A_wo, B_x, B_w1, B_w2):
    def _A_ref(x, wqkv, wo):
        B, S, D = x.shape
        H = 32; Dh = D // H; W = 256
        qkv = (lambda x, *d: x.transpose(*d))((x @ wqkv).reshape(B, S, 3, H, Dh), 2, 0, 3, 1, 4)
        q, k, v = qkv[0], qkv[1], qkv[2]
        scores = jnp.einsum("bhqd,bhkd->bhqk", q, k) * (Dh ** -0.5)
        idx = jnp.arange(S)
        mask = (idx[:, None] - idx[None, :] >= 0) & (idx[:, None] - idx[None, :] < W)
        scores = jnp.where(mask[None, None], scores, -1e9)
        p = _softmax(scores, axis=-1)
        o = jnp.einsum("bhqk,bhkd->bhqd", p, v)
        return (lambda x, *d: x.transpose(*d))(o, 0, 2, 1, 3).reshape(B, S, D) @ wo

    def _B_ref(x, w1, w2):
        h = jnp.einsum("bsd,df->bsf", x, w1)
        zero = jnp.zeros_like(h)
        h = jnp.maximum(h, zero)
        return jnp.einsum("bsf,fd->bsd", h, w2)

    x = A_x
    h = x + _A_ref(_layernorm(x, axis=-1), A_wqkv, A_wo)
    h2 = h + _B_ref(_layernorm(h, axis=-1), B_w1, B_w2)
    return h2
```

```python
from collections import Counter

import jax
import jax.numpy as jnp
import numpy as np
from jax import lax
from jax.experimental import pallas as pl
from jax.experimental.pallas import tpu as pltpu

S, D, DFF, H, DH = 2048, 640, 1536, 32, 20
EPS = 1e-5
T = 256
NB = S // T
F32, BF16, U32, I32 = jnp.float32, jnp.bfloat16, jnp.uint32, jnp.int32
QSCALE = float(DH ** -0.5 * np.log2(np.e))
MASKED = -1e30

UP_SCHEME = """
000000000000000+0000,00-00+000000000,000+--000+-- 0000000+000000000000,000000-00+00000,000-++000-++
000000000000000000+0,000000--0++0000,0000+00000+0 000000+0000000000000,0+-0-+000000000,0000-00000-0
000000+000000000-00+,0000+0000000000,0000000000-0 00000000-+00000000+0,0000000000+0000,0000-0000000
0000000-000000000+00,0000000+0000000,+0-000000-++ 0000000+0000000000+0,000000++0-00000,+0-0+0000-++
00000-000000000+0000,0+0000000000000,000+---0+000 000000+00000000+0000,0+-00+000000000,000-+++0-0+0
000000000+0000000000,0000000000+00+0,0+--+-+-0000 00000++0000000000000,0+-00000000+000,000+0--0+000
000+0--0-000000000+0,00000000000+000,00000-000000 000000000000000000+0,000000-0-+0+000,00000+00000+
0000000000000000000+,0000+00000000+0,0-+000-+0-+- 0+000000000000000000,000+++-0-0000++,00+00000000-
0+0000000000000++000,00000+000000000,00000000000+ 00000000000000000++0,000-00++0000000,-0+000000+0-
0-000000000000000++0,000-00+0+000000,+0-00000000+ 0+00000000000000000+,0000+00000000++,0+-00000000+
0000000++0000+000000,000000000+00000,000+00000000 000+0000000000000000,000000-0-+++0++,00+00+000000
000-00000+0000000000,0000000000+00++,0-+00+000000 000+000+0000000000+0,000000+0+-00000,-0+00+000000
+0+0000-000000000+00,00000000+000000,-0+000000000 000000+0000000000000,-0-+0+000000000,000+00000+00
+0000000000000000000,0--00000+000000,00-00000+000 -000+0000---0-+0000+,00000000000000+,0-+000000000
-000000000--0-+00000,0-000000000000+,0+-00000+000 0000000000--0-+00000,0+0000000000000,0+-0000-+000
00000--000000+000000,-0-00000000+000,000+00-0+000 000000000+000+000000,0000000000+0++0,000+00-+0000
0000000000000+000000,-0-000000+++++0,000-00+00000 0-0-+000000000000000,0000000+00000++,0+0000000000
00000000000-0000000+,0000+0000000++0,000000+-0+00 0+++-0000-00+0-0000+,000000000000+00,000000-+0000
0---+000000000000000,0000000+0000000,+-0000-+0000 0+++-0000000+0000000,0000000+0000-00,+00000-+0000
00000000000-0-+00000,0+0000000000++0,0000000+0000 000000000000+0000000,-00000++0000000,-00000+00000
00000000000+00000000,-0-+++000000++0,000000+00+00 -00000000000+0000000,+0000000+000000,-0000000+000
0+++00000000+0000000,000000+0+000+00,+00000000000 000000+0000+000+0000,-0-00+000000000,000000-0+-00
00000-0000-0-00+0000,+00000000000000,000000-0+000 000000-0000-0000+++0,000+00000000000,000000000+00
+000000000++0+000000,+0+00000000000+,00000000+000
"""
OUT_SCHEME = """
000-0000+0,000000000000000-0-0+00000,000000000+ 000-0+0000,00-0+0000000000+000000000,-00000000+
00000-00+0,00-00000000000-+000000000,00000+000+ 00000+0000,+-0000000000000+000000000,+0000+0000
+-000-+000,00000+0000000000000000000,00000++000 -+000+0000,0+000+0000000000000000000,+0000++000
+-00000000,0+00000000000000000000000,++000++000 0-00000000,0-0000-0+000000000000+000,0+00000000
00000000++,00+000000+0000000+0000000,0000000+0+ 00000-0++0,00000000000000+0000000000,00+++00+++
00+00+0--0,00+00000000000+0000000000,00+++-0++0 000000-0+0,000000000-000000+00000000,0+00+0+00+
000-000000,0000-0000-000000+00-0000+,0000+0000+ 000+00+0-0,0000000000000000+00000000,0+00+0000+
000+00000+,00-000000-0000000-000000+,00-000000+ 00+0000000,0000000000-000000000+0000,-0+00-0+00
00-0000+00,00+000000000+000000000000,00000-0+00 00-000000-,0000000000-0-0+00000+0000,00+00-0++0
0000000+0+,0000000000-0-0+0000000000,00000-00+0 000000+000,00000-++0-0-0000+00000000,000000+000
0-00-00000,000000000-00000000000+000,0-+000-+00 0-00-0+0-0,000000000+000000000000000,0-00-0-+00
0+00+0-00-,0000000-0+000000000000000,000000-+00 0+00+0000-,0000000+0-00000000000+000,00+000-+00
000000000+,00-000000--0-0+00-00+++00,00+0000+00 -0000+0000,-0--+-000000000000-0+00+0,+000000000
000000++00,00000000000+0000000000000,0+0+00+0+0 00+000--00,00000000-00+0000000000000,0+0+0000+0
0++000--00,00000000+0000000000000000,0+0+000000 +00-000000,00-0+00000000000000000000,+000+00000
+0-0+-0++0,00+000000000000000+000000,00+++000+0 -0++0+0--0,000000000000000000+000000,00+++00000
0000-0000+,0000000+0-000000000000-0+,00+0000000 -000-+000+,00000000000000000000+00+0,00000000+0
000++00000,00-000000-00000000-00000+,00+0+00000 +0+0+-0000,000-00000000000000-0+00+0,+0000000+0
00+0000-00,00000000+0-0--+000+000000,00000000+0 +000+00000,00-+000000000000000000000,000+0000+0
00-0000000,000-0000000+0-+000-0000+0,000+0000+0 00+0+00000,000-00000000000000-0000+0,-00+000000
"""
DOWN_SCHEME = """
+00000000000,00+0+0000000+00,0+++00000000+0000000 0+0000000000,0000000+0+0000+,0-0-+000000000000000
000000-+0000,0000+0000000000,0+++-0000-00+0-0000+ +00000-+0000,0000-00+0000000,0+++-0000000+0000000
+-0000-+0000,0000000+0000000,0---+000000000000000 00+00+000000,00-+0000++00-++,000+0000000000000000
-0+000000000,000000000000+00,+0+0000-000000000+00 -0000000+000,+00000000000+00,-00000000000+0000000
00000000+000,+000000000+000+,+000000000++0+000000 0-+000000000,00000000000000+,-000+0000---0-+0000+
0+-00000+000,00000-00000000+,-000000000--0-+00000 00-00000+000,00000-0000-0+00,+0000000000000000000
0+-0000-+000,00000+000000000,0000000000--0-+00000 0-+00+000000,00000000++0000+,000-00000+0000000000
0000000+0000,0000++000+00000,00000000000-0-+00000 -00000+00000,-0+0000+0000000,000000000000+0000000
000-00+00000,-00++000++-00+0,0000000000000+000000 000+00-+0000,0000+000++00000,000000000+000+000000
000000-0+000,+00000000000000,00000-0000-0-00+0000 0+--+-+-0000,00000000++00000,000000000+0000000000
0000-0000000,00000000+000000,00000000-+00000000+0 0+-00000000+,000000+00+0000+,0+00000000000000000+
000+00-0+000,-000000000-00+0,00000--000000+000000 00000-000000,0000000000000+0,000+0--0-000000000+0
000+00000000,000+00000000000,0000000++0000+000000 -0+00+000000,00+-00000000+00,000+000+0000000000+0
000000000+00,0+0000000000000,000000-0000-0000+++0 +0-0+0000-++,00+-000+0000000,0000000+0000000000+0
+0-000000-++,0000000+0000000,0000000-000000000+00 +0-00000000+,0-+000000000+00,0-000000000000000++0
-0+000000+0-,0-+0000+0000000,00000000000000000++0 00000+00000+,00-+00000000-+0,000000000000000000+0
0000+00000+0,00-+000-+000000,000000000000000000+0 00+00000000-,0+-000+00+0+-0+,0+000000000000000000
0000000000-0,000000+00000000,000000+000000000-00+ 00000000000+,00000000000+000,0+0000000000000++000
000+---0+000,00000+000000000,00000-000000000+0000 000-++000-++,00-+00000000000,0000000+000000000000
000+0--0+000,00000+0000-00+0,00000++0000000000000 000+--000+--,0000000000-+000,000000000000000+0000
0-+000-+0-+-,000000+00+00000,0000000000000000000+ 000000+-0+00,0000+0+00+00000,00000000000-0000000+
000000-0+-00,-000000000-+000,000000+0000+000+0000 000-+++0-0+0,00000+0000-+000,000000+00000000+0000
000000+00+00,-+00+0+00+-+000,00000000000+00000000 000+00000+00,-+00000000-+000,000000+0000000000000
0000-00000-0,00000+-000-+000,000000+0000000000000
"""

QKV_CHUNKS = ((5, 1), (0, 1), (6, 1), (1, 1), (7, 3), (2, 3), (10, 3), (13, 2))
QKV_PARTS = ((5, 6, 7), (8, 9, 0), (1, 2, 3), (4, 10, 11), (12, 13, 14))
X1_AFTER = 6
COPIES_AHEAD = 4

CFG = dict(
    FIRST="D40+A12+A12+A12+D64+A12+D24+A12+D22+A12+A2+A12+P8+A2+A12+P8+A2+P8+A2+P8+A2+P4+A2+P12+A2+P8+A2+P62"
          "+O40+B177+E12+B3+E8+Q40+E74"
          "/g14,3,8,3/g30,10,25,3/g88,31,20,10/k77,63,10,17/k140,30,37,8/k176,83,35,15/a138,91,18,8"
          "/u294,118,27,32/o300,54,21,8/h301,59,12,16/w608,86,24,32/b436,145,30,8/e259,4,0,8/f597,8,0,4"
          "/d578,145,24,8",
    LOOP="P118+F47+A177+F30+A3+F18+O40+E94"
         "/b0,88,14,6/g48,79,40,16/e352,22,6,4/b361,34,32,2/a435,85,16,8",
    LAST="F94+E94+G94"
         "/b0,66,24,8/s94,0,0,1",
    PV_LAG=5,
    EXP_AT=(0, 3, 7, 15),
    EXP_AT0=(0, 3, 9, 12, 4, 8, 7, 8),
)


def _cse(rows, nvar):
    rows = [dict(r) for r in rows]
    temps = []
    while True:
        cnt = Counter()
        for r in rows:
            ks = sorted(r)
            for x, a in enumerate(ks):
                for b in ks[x + 1:]:
                    cnt[a, b, r[a] * r[b]] += 1
        best = max(sorted(cnt.items()), key=lambda t: t[1], default=(None, 0))
        if best[1] < 2:
            return temps, rows
        a, b, sign = best[0]
        for r in rows:
            if a in r and b in r and r[a] * r[b] == sign:
                r[nvar + len(temps)] = r.pop(a)
                r.pop(b)
        temps.append((a, b, sign))


def _parse(m, k, n, text):
    words = [[{i: 1 if ch == "+" else -1 for i, ch in enumerate(f) if ch != "0"} for f in p.split(",")]
             for p in text.split()]
    u, v, w = ([p[i] for p in words] for i in range(3))
    for rows, nvar in ((u, m * k), (v, k * n)):
        for r, row in enumerate(_cse(rows, nvar)[1]):
            if max(row.values()) < 0:
                for f in (rows, w):
                    f[r] = {i: -c for i, c in f[r].items()}
    return u, v, w


def _halve(rows):
    m = len(rows)
    perm = list(range(m))

    def cost():
        return sum(len(set().union(*[rows[r] for r in g])) ** 2 for g in (perm[:m // 2], perm[m // 2:]))

    best, moved = cost(), True
    while moved:
        moved = False
        for a in range(m):
            for b in range(a + 1, m):
                perm[a], perm[b] = perm[b], perm[a]
                c = cost()
                if c < best:
                    best, moved = c, True
                else:
                    perm[a], perm[b] = perm[b], perm[a]
    return perm[:m // 2], perm[m // 2:]


def _signed_sum(terms):
    terms = sorted(terms, key=lambda t: -t[0])
    sign, acc = terms[0]
    for s, v in terms[1:]:
        acc = acc + v if s == sign else acc - v
    return sign, acc


def _sums(rows, nvar, block):
    temps, rows = _cse(rows, nvar)
    val = {}

    def get(x):
        if x not in val:
            if x < nvar:
                val[x] = (1, block(x))
            else:
                a, b, sign = temps[x - nvar]
                val[x] = _signed_sum([get(a), (get(b)[0] * sign, get(b)[1])])
        return val[x]

    return lambda r: _signed_sum([(c * get(x)[0], get(x)[1]) for x, c in sorted(rows[r].items())])


def _products(w, nout, mul, init, done, rows_per_product):
    nr = len(w)
    temps, rows = _cse([{r: x[c] for r, x in enumerate(w) if c in x} for c in range(nout)], nr)
    val, acc = {}, {}
    left = [len(r) for r in rows]
    for r in range(nr):
        val[r] = mul(r)
        new = [r]
        for t, (a, b, sign) in enumerate(temps):
            if nr + t not in val and a in val and b in val:
                val[nr + t] = _signed_sum([val[a], (val[b][0] * sign, val[b][1])])
                new.append(nr + t)
        for c, row in enumerate(rows):
            for x in new:
                if x in row:
                    terms = [(val[x][0] * row[x], val[x][1])]
                    if c in acc:
                        terms = [acc[c]] + terms
                    elif init is not None:
                        terms = [(1, init(c))] + terms
                    acc[c] = _signed_sum(terms)
                    left[c] -= 1
                    if not left[c]:
                        sign, v = acc.pop(c)
                        done(c, v if sign > 0 else -v)
        yield rows_per_product


def _layernorm(x):
    xc = x - jnp.mean(x, axis=-1, keepdims=True)
    return xc * lax.rsqrt(jnp.mean(xc * xc, axis=-1, keepdims=True) + EPS)


def _iota(shape, axis):
    return lax.broadcasted_iota(I32, shape, axis)


def _at(i, n=128):
    return pl.ds(pl.multiple_of(i, n), n)


def _make_kernel(cfg):
    up_scheme, out_scheme = _parse(4, 5, 3, UP_SCHEME), _parse(2, 5, 5, OUT_SCHEME)
    down_scheme = _parse(4, 3, 5, DOWN_SCHEME)

    def kernel(x_hbm, wqkv_hbm, wo_hbm, w1_hbm, w2_hbm, o_hbm,
               x_s, wqkv_s, wo_s, w1_s, w2_s, krep_s, vt_s, qt_s, o_s, p_s, h_s, out_s, hid_s, isem, osem,
               xc_s, hc_s, x0_s, k_s, co_s, *tiles):
        qkv_strips = {c0 + c: (buf, c) for (c0, n), buf in zip(QKV_CHUNKS, wqkv_s) for c in range(n)}
        cq_s, c1_s, c2_s = tiles[0:5], tiles[5:9], tiles[9:13]
        step = pl.program_id(0)

        zero = step >> 4
        never = zero > 0
        latest = []
        due = []
        clock = dict(now=0, slack=0)
        written = Counter()

        def matmul(a, b):
            r = jnp.dot(a, b, preferred_element_type=F32)
            latest[:] = [r[0:16, 0:128]]
            return r

        def must_finish(value):
            due.append((clock["now"] + clock["slack"], value))

        def after_due(w):
            due.sort(key=lambda t: t[0])
            while due and due[0][0] <= clock["now"]:
                w = jnp.concatenate([jnp.where(never, due.pop(0)[1], w[0:8]), w[8:]], axis=0)
            return w

        def run(plan, streams, jobs):
            order, *specs = plan.split("/")
            clock["now"] = 0
            todo = []
            for spec in specs:
                start, span, slack, steps = (int(v) for v in spec[1:].split(","))
                steps *= 2 if spec[0] in "kouw" else 1
                todo += [(128 * start + 128 * span * i // steps, 128 * slack, jobs[spec[0]]) for i in range(steps)]
            todo.sort(key=lambda t: t[0])
            for item in order.split("+"):
                end = clock["now"] + 128 * int(item[1:])
                while clock["now"] < end:
                    rows = next(streams[item[0]], None)
                    if rows is None:
                        break
                    clock["now"] += rows
                    while todo and todo[0][0] <= clock["now"]:
                        _, clock["slack"], job = todo.pop(0)
                        next(job, None)
            assert not todo and all(next(g, None) is None for g in (*streams.values(), *jobs.values()))
            due.clear()
            latest.clear()

        def packed(ref, i, n, first=0):
            return ref.bitcast(U32)[i, first:first + n, :]

        def operand(ref, i, rows=128, first_row=0, whole=None):
            assert written[id(ref), i] == (whole or rows // 16)
            return pltpu.bitcast(after_due(packed(ref, i, rows // 2, first_row // 2)), BF16)

        def store_sums(dst, which, row, c):
            for i, r in enumerate(which):
                sign, v = row(i)
                dst[r, 16 * c:16 * c + 16, :] = (v if sign > 0 else -v).astype(BF16)
                written[id(dst), r] = c + 1
            must_finish(packed(dst, zero + which[0], 8))

        def norm_sums(load, dst):
            for c in range(4):
                xn = []
                for i in range(4):
                    x = load(64 * i + 16 * c)
                    if latest:
                        x = jnp.concatenate([jnp.where(never, latest[0], x[:, 0:128]), x[:, 128:]], axis=1)
                    xn.append(_layernorm(x))
                    if i == 1:
                        yield 1
                row = _sums(up_scheme[0], 20, lambda b: xn[b // 5][:, 128 * (b % 5):128 * (b % 5) + 128])
                store_sums(dst, range(47), row, c)
                yield 1

        def norm1(j):
            return norm_sums(lambda r: x_s[_at(j * T + r, 16), :].astype(F32), xc_s)

        def norm2(j):
            assert written["h"]
            yield from norm_sums(lambda r: h_s[j, r:r + 16, :], hc_s)

        def place(src, k, c):
            if src is w2_hbm:
                return w2_s, 4 * c + k // 3, 128 * (k % 3)
            buf, i = qkv_strips[c] if src is wqkv_hbm else (wo_s, c) if src is wo_hbm else (w1_s[c // 6], c % 6)
            return buf, i, 128 * k

        def raw_tile(src, k, c):
            buf, i, r = place(src, k, c)
            return operand(buf, i, first_row=r, whole=40)

        def weights(v, src, row_tiles, col_tiles, dst):
            n = len(col_tiles)
            keys = [tuple(sorted(row.items())) for row in v]
            sums = [r for r, key in enumerate(keys) if len(key) > 1 and keys.index(key) == r]

            def get(r):
                if len(keys[r]) > 1:
                    return operand(dst, keys.index(keys[r]))
                (b, sign), = keys[r]
                assert sign > 0
                return raw_tile(src, row_tiles[b // n], col_tiles[b % n])

            def job():
                halves = [[sums[i] for i in half] for half in _halve([v[r] for r in sums])]
                for c in range(8):
                    for q, which in enumerate(halves):
                        def block(b):
                            buf, i, r = place(src, row_tiles[b // n], col_tiles[b % n])
                            return buf[i, _at(r + 16 * c + 16 * (zero >> q), 16), :].astype(F32)

                        store_sums(dst, which, _sums([v[r] for r in which], len(row_tiles) * n, block), c)
                        yield 1

            return get, job()

        qkv_w = [weights(up_scheme[1], wqkv_hbm, range(5), cols, dst) for cols, dst in zip(QKV_PARTS, cq_s)]
        out_w = weights(out_scheme[1], wo_hbm, range(5), range(5), co_s)
        up_w = [weights(up_scheme[1], w1_hbm, range(5), range(3 * i, 3 * i + 3), c1_s[i]) for i in range(4)]
        down_w = [weights(down_scheme[1], w2_hbm, range(3 * i, 3 * i + 3), range(5), c2_s[i]) for i in range(4)]

        def keep(j, part, c, val):
            i, c = divmod(c, 5)
            if part == 0:
                qt_s[2 * j + i, 64 * c:64 * c + 64, :] = pltpu.bitcast((val * QSCALE).astype(BF16).T, U32)
            elif part == 1:
                assert not isinstance(j, int) or j == 0 or written["rep", id(j - 1), H - 1]
                k_s[5 * i + c, 0:128, :] = val.astype(BF16)
            else:
                val, low = val.T, _iota((8, 128), 0) < 4
                for n in range(16):
                    pair, e = divmod(16 * c + n, 5)
                    x = val[8 * n:8 * n + 8]
                    r = 48 * pair + 8 * (e + (e > 2))
                    if e == 2:
                        vt_s[2 * j + i, r:r + 8, :] = jnp.where(low, x, 1.0)
                        vt_s[2 * j + i, r + 8:r + 16, :] = jnp.where(low, 1.0, x)
                    else:
                        vt_s[2 * j + i, r:r + 8, :] = x
            written["qkv"[part], id(j), i, c] = 1

        def project(j):
            for part, cols in enumerate(QKV_PARTS):
                out = {}

                def done(c, val):
                    i, n = divmod(c, 3)
                    out[i, n] = val
                    if (i ^ 1, n) in out:
                        keep(j, cols[n] // 5, 5 * (i // 2) + cols[n] % 5,
                             jnp.concatenate([out[i & 2, n], out[i | 1, n]], axis=0))

                yield from _products(up_scheme[2], 12,
                                     lambda r: (1, matmul(operand(xc_s, r, 64), qkv_w[part][0](r))),
                                     None, done, 64)

        def spread_keys(j):
            for h in range(H):
                c, off = divmod(DH * h, 128)
                for i in range(2):
                    assert written["k", id(j), i, c] and written["k", id(j), i, (DH * h + DH - 1) // 128]
                    src = packed(k_s, 5 * i + c, 64)
                    if off + DH > 128:
                        src = jnp.where(_iota((64, 128), 1) >= off, src, packed(k_s, 5 * i + c + 1, 64))
                    lanes = ((_iota((8, 128), 1) & 31) + off) & 127
                    krep_s[h, _at(64 * (2 * j + i), 64), :] = jnp.take_along_axis(
                        src, jnp.concatenate([lanes] * 8, axis=0), axis=1)
                written["rep", id(j), h] = 1
                if h % 2:
                    must_finish(krep_s[zero + h, 0:8, :])
                    yield 1

        def masks():
            r2, c2 = 2 * _iota((64, 128), 0), _iota((64, 128), 1)
            return (_iota((128, 128), 0) > _iota((128, 128), 1),
                    jnp.where(r2 > c2, jnp.uint32(0xFFFF), jnp.uint32(0))
                    | jnp.where(r2 + 1 > c2, jnp.uint32(0xFFFF0000), jnp.uint32(0)))

        def attention(j, first, upper, upper_packed):
            group = _iota((16, 128), 1) >> 5

            def scores(h, b):
                assert written["rep", id(j), h] and written["q", id(j), b, (DH * h + DH - 1) // 128]
                assert written["q", id(j), b, DH * h // 128]
                q = qt_s[2 * j + b, pl.ds(10 * h, 16), :]
                q = [jnp.where((group == g) & (_iota((16, 128), 0) < 10), q, jnp.uint32(0)) for g in range(4)]
                q = pltpu.bitcast(jnp.concatenate(q, axis=0), BF16)
                if first:
                    raw = matmul(pltpu.bitcast(krep_s[h, 0:64 * (b + 1), :], BF16), q)
                    s = jnp.where(upper, MASKED, raw[128 * b:128 * b + 128])
                    s = jnp.concatenate([raw[0:128], s], axis=0) if b else s
                else:
                    k = krep_s[h, pl.ds(pl.multiple_of(64 * (2 * j + b - 2), 64), 192), :]
                    k = [k[16 * n:16 * n + 16] for n in range(12)]
                    k = k[3:9] + [jnp.where(group <= n, k[n], k[n + 9]) for n in range(3)]
                    raw = matmul(pltpu.bitcast(jnp.concatenate(k, axis=0), BF16), q)
                    oldest = jnp.concatenate([raw[192:288], raw[0:32]], axis=0)
                    s = jnp.concatenate([jnp.where(upper, oldest, raw[160:288]), raw[32:160]], axis=0)
                return raw, s, jnp.max(s, axis=0, keepdims=True)

            def weigh(h, b):
                assert all(written["v", id(j), i, c] for i in range(2) for c in range(5))
                p = after_due(packed(p_s, b * H + h, 64 * (b + 1) if first else 128))
                if first:
                    tiles_ = range(b + 1)
                else:
                    oldest = p[0:64] & upper_packed
                    p = jnp.concatenate([oldest, p[64:128], p[0:64] ^ oldest], axis=0)
                    tiles_ = [2 * j + b - 2 + n for n in range(3)]
                v = jnp.concatenate([vt_s[t, 24 * h:24 * h + 24, :] for t in tiles_], axis=1)
                return jnp.dot(v, pltpu.bitcast(p, BF16), preferred_element_type=F32)

            if first:
                groups = [[(h, b) for b in (1, 0) for h in range(h0, h0 + 4)] for h0 in range(0, H, 4)]
            else:
                groups = [[(h, b) for h in range(h0, h0 + 4)] for b in range(2) for h0 in range(0, H, 4)]
            pending = {}

            def exps(tiles_, raw):
                for i, (h, b) in enumerate(tiles_):
                    s, m = pending.pop((h, b))
                    r = 8 * cfg["EXP_AT0" if first else "EXP_AT"][i]
                    m = jnp.where(never, raw[i][r:r + 1] if raw else latest[0][0:1], m)
                    p_s[b * H + h, 0:s.shape[0], :] = jnp.exp2(s - m).astype(BF16)
                    yield 1

            def stream():
                lag = cfg["PV_LAG"] if first else 1
                low = _iota((8, 128), 0) < 4
                rows = ([], [])
                for new, mid, old in zip(groups + [[]] * lag, [[]] + groups + [[]] * lag, [[]] * lag + groups):
                    if new:
                        raw = []
                        for h, b in new:
                            r, *pending[h, b] = scores(h, b)
                            raw.append(r)
                        for _ in exps(mid, raw):
                            pass
                        yield sum(r.shape[0] for r in raw)
                    assert not any(t in pending for t in old)
                    for (h, b), odd in zip(old[0::2], old[1::2]):
                        e, o = weigh(h, b), weigh(*odd)
                        inv = pl.reciprocal(jnp.where(low, o[0:8], e[16:24]), approx=True)
                        swapped = pltpu.roll(inv, 4, 0)
                        ie, io = jnp.where(low, swapped, inv), jnp.where(low, inv, swapped)
                        rows[b].extend([e[0:8] * ie, e[8:16] * ie, jnp.where(low, e[16:24], o[0:8]) * swapped,
                                        o[8:16] * io, o[16:24] * io])
                        if len(rows[b]) >= 16:
                            c = 5 * b + (DH * h + 2 * DH) // 128 - 1
                            o_s[j, c] = jnp.concatenate(rows[b][:16], axis=0).T
                            written["o", id(j), c] = 1
                            del rows[b][:16]
                    if old:
                        yield 288

            return stream(), exps(groups[-1], None)

        def out_proj(j):
            assert all(written["o", id(j), c] for c in range(10))
            a = _sums(out_scheme[0], 10, lambda c: o_s[j, c])

            def mul(r):
                sign, val = a(r)
                return sign, matmul(val, out_w[0](r))

            def done(c, val):
                h_s[j, 128 * (c // 5):128 * (c // 5) + 128, 128 * (c % 5):128 * (c % 5) + 128] = val

            for n, rows in enumerate(_products(
                    out_scheme[2], 10, mul,
                    lambda c: x_s[_at(j * T + 128 * (c // 5)), 128 * (c % 5):128 * (c % 5) + 128].astype(F32),
                    done, 128)):
                written["h"] += n == 39
                yield rows

        def ffn_up():
            for part in range(4):
                def done(c, val):
                    hid_s[3 * part + c % 3, 64 * (c // 3):64 * (c // 3) + 64, :] = jnp.maximum(val, 0.0)

                yield from _products(up_scheme[2], 12,
                                     lambda r: (1, matmul(operand(hc_s, r, 64), up_w[part][0](r))),
                                     None, done, 64)

        def ffn_down(j, sent=None):
            a = _sums(down_scheme[0], 12, lambda c: jnp.concatenate(
                [hid_s[3 * part + c % 3, 64 * (c // 3):64 * (c // 3) + 64, :] for part in range(4)], axis=1))
            ready = set()

            def mul(r):
                sign, val = a(r)
                return sign, matmul(val, jnp.concatenate([w[0](r) for w in down_w], axis=0))

            def done(c, val):
                i, n = divmod(c, 5)
                out_s[_at(j * T + 64 * i, 64), 128 * n:128 * n + 128] = val.astype(out_s.dtype)
                ready.add((i, n))
                if sent is not None and (i ^ 1, n) in ready:
                    where = (pl.ds(j * T + 64 * (i & 2), 128), pl.ds(128 * n, 128))
                    sent.append(pltpu.make_async_copy(out_s.at[where], o_hbm.at[where], osem))
                    sent[-1].start()

            return _products(
                down_scheme[2], 20, mul,
                lambda c: h_s[j, 64 * (c // 5):64 * (c // 5) + 64, 128 * (c % 5):128 * (c % 5) + 128],
                done, 256)

        def send(j):
            return pltpu.make_async_copy(out_s.at[_at(j * T, T)], o_hbm.at[_at(j * T, T)], osem)

        def strips(src, cols):
            n = 3 if src is w2_hbm else 5
            at = [(k, c, *place(src, k, c)) for c in cols for k in range(0, src.shape[0] // 128, n)]
            return [(src.at[pl.ds(128 * k, 128 * n), pl.ds(128 * c, 128)], buf.at[i, pl.ds(0, 128 * n)], (id(buf), i))
                    for k, c, buf, i, _ in at]

        copies = {"x0": [(x_hbm.at[0:T], x_s.at[0:T], None)]}
        for i, (c, n) in enumerate(QKV_CHUNKS):
            if i == X1_AFTER:
                copies["x1"] = [(x_hbm.at[T:2 * T], x_s.at[T:2 * T], None)]
            copies[c] = strips(wqkv_hbm, range(c, c + n))
        for i in range(2):
            copies["w1", i] = strips(w1_hbm, range(6 * i, 6 * i + 6))
        copies["wo"] = strips(wo_hbm, range(5))
        copies["w2"] = strips(w2_hbm, range(5))
        copies["x"] = [(x_hbm.at[2 * T:S], x_s.at[2 * T:S], None)]
        names = list(copies)

        def fetch(i, offset=0):
            sem = isem.at[i % (COPIES_AHEAD + 2) + offset]
            return [pltpu.make_async_copy(src, dst, sem) for src, dst, _ in copies[names[i]]]

        def arrived(name, then):
            while written["copies"] < names.index(name):
                written["copies"] += 1
                i = written["copies"]
                here = jnp.where(never, pltpu.bitcast(latest[0][0:8], I32), 0)[0, 0]
                for copy in fetch(i, here):
                    copy.wait()
                written.update({key: 40 for _, _, key in copies[names[i]]})
                if i + COPIES_AHEAD < len(names):
                    for copy in fetch(i + COPIES_AHEAD, here):
                        copy.start()
            yield from then

        def in_sequence(jobs):
            for job in jobs:
                yield from job

        def in_turn(jobs):
            for _ in range(8):
                for job in jobs:
                    yield next(job)
                    yield next(job)

        def first():
            mask = masks()
            fetch(0)[0].wait()
            for c in range(T // 16):
                xn = _layernorm(x_s[16 * c:16 * c + 16, :].astype(F32))
                for k in range(5):
                    x0_s[5 * (c // 8) + k, 16 * (c % 8):16 * (c % 8) + 16, :] = (
                        xn[:, 128 * k:128 * k + 128].astype(BF16))
                    written[id(x0_s), 5 * (c // 8) + k] = 8
            latest[:] = [xn[:, 0:128]]

            def project_directly():
                left = 75
                for c0, n in QKV_CHUNKS:
                    yield from arrived(c0, ())
                    for c in range(c0, c0 + n):
                        for k in range(5):
                            a = jnp.concatenate([operand(x0_s, k), operand(x0_s, 5 + k)], axis=0)
                            w = raw_tile(wqkv_hbm, k, c)
                            if left < 4:
                                r = jnp.concatenate([matmul(a[64 * i:64 * i + 64], w) for i in range(4)], axis=0)
                            else:
                                r = matmul(a, w)
                            left -= 1
                            acc = acc + r if k else r
                            if k == 4:
                                for i in range(2):
                                    keep(0, c // 5, 5 * i + c % 5, acc[128 * i:128 * i + 128])
                            yield 256

            a0, tail0 = attention(0, True, *mask)
            a1, tail1 = attention(1, False, *mask)
            streams = dict(D=project_directly(), A=a0, P=project(1), O=out_proj(0), B=a1, E=ffn_up(), Q=out_proj(1))
            jobs = dict(
                a=arrived("x1", norm1(1)), b=norm2(0), d=arrived("x", norm1(2)), e=tail0, f=tail1,
                g=spread_keys(0), h=spread_keys(1),
                k=in_sequence([arrived(chunk, w[1]) for chunk, w in zip((7, 7, 2, 10, 13), qkv_w)]),
                o=arrived("wo", out_w[1]),
                u=in_turn([arrived(("w1", i // 2), w[1]) for i, w in enumerate(up_w)]),
                w=in_turn([arrived("w2", w[1]) for w in down_w]))
            run(cfg["FIRST"], streams, jobs)

        def rest():
            mask = masks()

            def block(j):
                a, tail = attention(j, False, *mask)
                written.update({(id(hc_s), r): -4 for r in range(47)})
                run(cfg["LOOP"],
                    dict(P=project(j), F=ffn_down(j - 2), A=a, O=out_proj(j), E=ffn_up()),
                    dict(a=norm1(jnp.minimum(j + 1, NB - 1)), b=norm2(j - 1), e=tail, g=spread_keys(j)))
                send(j - 2).start()

            pl.loop(2, NB)(block)
            sent = []

            def send_previous():
                send(NB - 2).start()
                yield 1

            written.update({(id(hc_s), r): -4 for r in range(47)})
            run(cfg["LAST"], dict(F=ffn_down(NB - 2), E=ffn_up(), G=ffn_down(NB - 1, sent)),
                dict(b=norm2(NB - 1), s=send_previous()))
            for copy in [send(j) for j in range(NB - 1)] + sent:
                copy.wait()

        later = zero
        for i in range(COPIES_AHEAD + 1):
            pl.when(step < 1)(fetch(i, later if i else 0)[0].start)
            for _ in range(2 if i else 8):
                later = later * later
        pl.when(step == 0)(first)
        pl.when(step == 1)(rest)

    return kernel


@jax.jit
def pallas_sequential_preLN__sliding_block__dense_activation_relu__prompt_kernel(
        A_x, A_wqkv, A_wo, B_x, B_w1, B_w2):
    del B_x
    hbm = pl.BlockSpec(memory_space=pl.ANY)
    out = pl.pallas_call(
        _make_kernel(CFG),
        grid=(2,),
        in_specs=[hbm] * 5,
        out_specs=hbm,
        out_shape=jax.ShapeDtypeStruct((S, D), A_x.dtype),
        scratch_shapes=[
            pltpu.VMEM((S, D), A_x.dtype),
            [pltpu.VMEM((n, D + 16, 128), BF16) for _, n in QKV_CHUNKS],
            pltpu.VMEM((5, D + 16, 128), BF16),
            [pltpu.VMEM((6, D + 16, 128), BF16)] * 2,
            pltpu.VMEM((20, DFF // 4 + 16, 128), BF16),
            pltpu.VMEM((H, S // 2, 128), U32),
            pltpu.VMEM((S // 128, H * 24, 128), F32),
            pltpu.VMEM((S // 128, D // 2 + 8, 128), U32),
            pltpu.VMEM((NB, 10, 128, 128), F32),
            pltpu.VMEM((2 * H, 256, 128), BF16),
            pltpu.VMEM((NB, T, D), F32),
            pltpu.VMEM((S, D), A_x.dtype),
            pltpu.VMEM((12, T + 8, 128), F32),
            pltpu.SemaphoreType.DMA((COPIES_AHEAD + 2,)),
            pltpu.SemaphoreType.DMA(()),
            *[pltpu.VMEM((47, 80, 128), BF16)] * 2,
            *[pltpu.VMEM((n, 144, 128), BF16) for n in (10, 10, 40) + (47,) * 13],
        ],
        compiler_params=pltpu.CompilerParams(
            dimension_semantics=("arbitrary",),
            vmem_limit_bytes=100 * 1024 * 1024,
            flags={"XLA_TPU_RESCHEDULE_DMA_DONES": True,
                   "XLA_TPU_EVENLY_DISTRIBUTE_CRITICAL_NODES": True}),
        name="fused_block",
    )(A_x.reshape(S, D), A_wqkv, A_wo, B_w1, B_w2)
    return out.reshape(A_x.shape)
```
